```python
import os as _os
_os.environ.setdefault("JAX_PLATFORMS", "cpu")
import jax
import jax.numpy as jnp

def _softmax(x, axis=-1):
    return jax.nn.softmax(x, axis=axis)
def _gelu(x):
    return jax.nn.gelu(x, approximate=True)
def _silu(x):
    return jax.nn.silu(x)
def _sigmoid(x):
    return jax.nn.sigmoid(x)
def _layernorm(x, axis=-1, eps=1e-5):
    m = jnp.mean(x, axis=axis, keepdims=True)
    v = jnp.var(x, axis=axis, keepdims=True)
    return (x - m) / jnp.sqrt(v + eps)
def _scatter_add(tgt, idx, src, axis=0):
    return tgt.at[idx].add(src)
def _segment_sum(src, seg, n):
    return jax.ops.segment_sum(src, seg, n)
class _Rng:
    def __init__(self, key):
        self._k = key
    def _next(self):
        self._k, sub = jax.random.split(self._k)
        return sub
    def normal(self, shape):
        return jax.random.normal(self._next(), shape, dtype=jnp.bfloat16)
    def randint(self, lo, hi, shape):
        return jax.random.randint(self._next(), shape, lo, hi, dtype=jnp.int32)
    def uniform(self, shape, lo=0.0, hi=1.0):
        return jax.random.uniform(self._next(), shape, jnp.bfloat16, lo, hi)
    def permutation(self, n):
        return jax.random.permutation(self._next(), n)


kernel_name = 'concat_heads__gqa_block_cached__mha_block_cached__near_ridge'

def setup_inputs():
    _rng = _Rng(jax.random.key(int.from_bytes(__import__("os").urandom(4), "little")))
    _w = (lambda a: (lambda t: t.astype(jnp.bfloat16) if jnp.issubdtype(t.dtype, jnp.floating) else t)(jnp.asarray(a)))
    def _A_setup():
        B, Sq, D = 16, 32, 1024
        Hq, Hkv, Sk, Dh = 32, 4, 32, 128
        assert Hq % Hkv == 0, (Hq, Hkv)
        return {
            "x": _w((lambda *s: _rng.normal(s) * 0.8)(B, Sq, D)),
            "k_cache": _w((lambda *s: _rng.normal(s) * 0.8)(B, Hkv, Sk, Dh)),
            "v_cache": _w((lambda *s: _rng.normal(s) * 0.05)(B, Hkv, Sk, Dh)),
            "wq": _w((lambda *s: _rng.normal(s) * 0.8)(D, Hq * Dh) * (D ** -0.5)),
            "wo": _w((lambda *s: _rng.normal(s) * 0.05)(Hq * Dh, D) * ((Hq * Dh) ** -0.5)),
        }
    _A_in = _A_setup()

    def _B_setup():
        B, Sq, D = 16, 32, 1024
        H, Sk, Dh = 32, 32, 128
        return {
            "x": _w((lambda *s: _rng.normal(s) * 0.8)(B, Sq, D)),
            "k_cache": _w((lambda *s: _rng.normal(s) * 0.8)(B, H, Sk, Dh)),
            "v_cache": _w((lambda *s: _rng.normal(s) * 0.05)(B, H, Sk, Dh)),
            "wq": _w((lambda *s: _rng.normal(s) * 0.8)(D, H * Dh) * (D ** -0.5)),
            "wo": _w((lambda *s: _rng.normal(s) * 0.05)(H * Dh, D) * ((H * Dh) ** -0.5)),
        }
    _B_in = _B_setup()

    return {
        "A_x": _A_in["x"],
        "A_k_cache": _A_in["k_cache"],
        "A_v_cache": _A_in["v_cache"],
        "A_wq": _A_in["wq"],
        "A_wo": _A_in["wo"],
        "B_x": _B_in["x"],
        "B_k_cache": _B_in["k_cache"],
        "B_v_cache": _B_in["v_cache"],
        "B_wq": _B_in["wq"],
        "B_wo": _B_in["wo"],
    }

def reference(A_x, A_k_cache, A_v_cache, A_wq, A_wo, B_x, B_k_cache, B_v_cache, B_wq, B_wo):
    def _A_ref(x, k_cache, v_cache, wq, wo):
        B, Sq, D = x.shape
        Hq, Dh = 32, 128
        Hkv = k_cache.shape[1]
        rep = Hq // Hkv
        q = (lambda x, *d: x.transpose(*d))((x @ wq).reshape(B, Sq, Hq, Dh), 0, 2, 1, 3)
        k = jnp.repeat(k_cache, rep, axis=1)
        v = jnp.repeat(v_cache, rep, axis=1)
        scores = jnp.einsum("bhqd,bhkd->bhqk", q, k) * (Dh ** -0.5)
        p = _softmax(scores, axis=-1)
        o = jnp.einsum("bhqk,bhkd->bhqd", p, v)
        return (lambda x, *d: x.transpose(*d))(o, 0, 2, 1, 3).reshape(B, Sq, Hq * Dh) @ wo

    def _B_ref(x, k_cache, v_cache, wq, wo):
        B, Sq, D = x.shape
        H, Dh = 32, 128
        q = (lambda x, *d: x.transpose(*d))((x @ wq).reshape(B, Sq, H, Dh), 0, 2, 1, 3)
        scores = jnp.einsum("bhqd,bhkd->bhqk", q, k_cache) * (Dh ** -0.5)
        p = _softmax(scores, axis=-1)
        o = jnp.einsum("bhqk,bhkd->bhqd", p, v_cache)
        return (lambda x, *d: x.transpose(*d))(o, 0, 2, 1, 3).reshape(B, Sq, H * Dh) @ wo

    a = _A_ref(A_x, A_k_cache, A_v_cache, A_wq, A_wo)
    b = _B_ref(B_x, B_k_cache, B_v_cache, B_wq, B_wo)
    return jnp.concatenate([a, b], axis=-1)
```

```python
import functools
import jax
import jax.numpy as jnp
from jax import lax
from jax.experimental import pallas as pl
from jax.experimental.pallas import tpu as pltpu

NB, SQ, D = 16, 32, 1024
H, DH, SK = 32, 128, 32
HKV = 4
M = NB * SQ
G = 4
NS = H // G
CW = G * DH
JB = 4
NJ = NB // JB
KQ = D // 4
SCALE = DH ** -0.5
LOG2E = 1.4426950408889634
NT = (((1,), (1,)), ((), ()))
TN = (((0,), (0,)), ((), ()))
F32 = jnp.float32
BF = jnp.bfloat16
OC = 256
NOUT = 1 + D // OC + 1


def _kernel(xa_h, ka_h, va_h, wqa_h, woa_h, xb_h, kb_h, vb_h, wqb_h, wob_h, out_h,
            x_v, wq_v, wo_v, ka_v, va_v, kb_v, vb_v, q_v, qp_v, acc_v, ob_v, sem_out):
    wq_h = (wqa_h, wqb_h)
    wo_h = (woa_h, wob_h)
    cp = pltpu.make_async_copy

    def out_copies():
        cs = [cp(ob_v.at[0], out_h.at[:, pl.ds(0, D)], sem_out.at[0])]
        for c in range(D // OC - 1):
            cs.append(cp(ob_v.at[1, :, pl.ds(c * OC, OC)], out_h.at[:, pl.ds(D + c * OC, OC)], sem_out.at[1 + c]))
        c = D // OC - 1
        for r in range(2):
            rows = pl.ds(r * (M // 2), M // 2)
            cs.append(cp(ob_v.at[1, rows, pl.ds(c * OC, OC)], out_h.at[rows, pl.ds(D + c * OC, OC)],
                         sem_out.at[1 + c + r]))
        return cs

    def main(sem_s, sem_step, bar):
        def barrier():
            pl.semaphore_signal(bar, 1)
            pl.semaphore_wait(bar, 1)

        def start_copies(s):
            if s < 4:
                ks = pl.ds(s * KQ, KQ)
                return [cp(xa_h.at[:, ks], x_v.at[0, :, ks], sem_s.at[s]),
                        cp(wqa_h.at[ks, pl.ds(0, CW)], wq_v.at[0, ks, :], sem_s.at[s])]
            hw = CW // 2
            if s == 4:
                h0 = pl.ds(0, 1)
                return [cp(ka_h.at[:, h0], ka_v.at[:, h0], sem_s.at[s]),
                        cp(va_h.at[:, h0], va_v.at[:, h0], sem_s.at[s]),
                        cp(wqa_h.at[:, pl.ds(CW, hw)], wq_v.at[1, :, pl.ds(0, hw)], sem_s.at[s])]
            return [cp(wqa_h.at[:, pl.ds(CW + hw, hw)], wq_v.at[1, :, pl.ds(hw, hw)], sem_s.at[s]),
                    cp(woa_h.at[pl.ds(0, CW), :], wo_v.at[0], sem_s.at[s])]

        def cp_wq(i, sem):
            if isinstance(i, int):
                return cp(wq_h[i // NS].at[:, pl.ds((i % NS) * CW, CW)], wq_v.at[i], sem)
            return cp(wqa_h.at[:, pl.ds(0, CW)], wq_v.at[i], sem)

        def cp_wo(blk, g, sem):
            return cp(wo_h[blk].at[pl.ds(g * CW, CW), :], wo_v.at[blk * NS + g], sem)

        def step_copies(blk, g):
            i = blk * NS + g
            sem = sem_step.at[i]
            cs = []
            if blk == 1:
                cs.append(cp(kb_h.at[:, pl.ds(g * G, G)], kb_v.at[g], sem))
                cs.append(cp(vb_h.at[:, pl.ds(g * G, G)], vb_v.at[g], sem))
            if not (isinstance(i, int) and i == 2 * NS - 1):
                cs.append(cp_wq(i + 1, sem))
            cs.append(cp_wo(blk, g, sem))
            return cs

        def kv_rest():
            hs = pl.ds(1, HKV - 1)
            return [cp(ka_h.at[:, hs], ka_v.at[:, hs], sem_step.at[2]),
                    cp(va_h.at[:, hs], va_v.at[:, hs], sem_step.at[2])]

        def cp_xb():
            return [cp(xb_h, x_v.at[1], sem_step.at[NS - 1])]

        for s in range(6):
            for c in start_copies(s):
                c.start()
            barrier()
        for i in range(1, 2 * NS):
            cs = step_copies(i // NS, i % NS)
            if i == 2:
                cs += kv_rest()
            if i == NS - 1:
                cs += cp_xb()
            for c in cs:
                c.start()
            if i < 2 * NS - 1:
                barrier()

        lane = lax.broadcasted_iota(jnp.int32, (SK, JB * SQ), 1)

        def qproj(xi, i, h):
            q_v[:, pl.ds(h * DH, DH)] = jnp.dot(x_v[xi], wq_v[i, :, pl.ds(h * DH, DH)],
                                                preferred_element_type=F32).astype(BF)

        def softmax_t(d):
            m = jnp.max(d, axis=0, keepdims=True)
            e = jnp.exp2((d - m) * (SCALE * LOG2E))
            l = jnp.sum(e, axis=0, keepdims=True)
            return (e * pl.reciprocal(l, full_range=False)).astype(BF)

        def load_q(h):
            return [q_v[pl.ds(j * JB * SQ, JB * SQ), pl.ds(h * DH, DH)] for j in range(NJ)]

        def qk(g, h, q):
            ps = []
            for j in range(NJ):
                ks = kb_v[g, pl.ds(j * JB, JB), h].reshape(JB * SK, DH)
                st = lax.dot_general(ks, q[j], NT, preferred_element_type=F32)
                d = st[(JB - 1) * SK:]
                for t in range(JB - 2, -1, -1):
                    d = jnp.where(lane < (t + 1) * SQ, st[t * SK:(t + 1) * SK], d)
                ps.append(softmax_t(d).T)
            return ps

        def pv(g, h, ps):
            os_ = []
            for j in range(NJ):
                for t in range(JB):
                    os_.append(jnp.dot(ps[j][t * SQ:(t + 1) * SQ], vb_v[g, j * JB + t, h],
                                       preferred_element_type=F32))
            return jnp.concatenate(os_, axis=0)

        def load_qt(j):
            return [jnp.concatenate([q_v[pl.ds(b * SQ, SQ), pl.ds(h * DH, DH)] for h in range(G)], axis=0)
                    for b in range(j * JB, (j + 1) * JB)]

        def qk_t(g, j, qs):
            c = g // (NS // HKV)
            return [softmax_t(lax.dot_general(ka_v[j * JB + t, c], qs[t], NT, preferred_element_type=F32))
                    for t in range(JB)]

        def pv_t(g, j, ps):
            c = g // (NS // HKV)
            os_ = []
            for t in range(JB):
                o = lax.dot_general(ps[t], va_v[j * JB + t, c], TN, preferred_element_type=F32)
                os_.append(jnp.concatenate([o[h * SQ:(h + 1) * SQ] for h in range(G)], axis=1))
            return jnp.concatenate(os_, axis=0)

        def att_q(blk, g):
            i1 = blk * NS + g + 1
            xi = i1 // NS
            f_load, f_qk, f_pv = (load_qt, qk_t, pv_t) if blk == 0 else (load_q, qk, pv)
            q = [f_load(t) for t in range(4)]
            qproj(xi, i1, 0)
            p0 = f_qk(g, 0, q[0])
            p1 = f_qk(g, 1, q[1])
            qproj(xi, i1, 1)
            p2 = f_qk(g, 2, q[2])
            p3 = f_qk(g, 3, q[3])
            o0 = f_pv(g, 0, p0)
            o1 = f_pv(g, 1, p1)
            qproj(xi, i1, 2)
            o2 = f_pv(g, 2, p2)
            o3 = f_pv(g, 3, p3)
            qproj(xi, i1, 3)
            return jnp.concatenate([o0, o1, o2, o3], axis=blk).astype(BF)

        def oproj(blk, g, o, first):
            for n in range(D // DH):
                cs = pl.ds(n * DH, DH)
                r = jnp.dot(o, wo_v[blk * NS + g, :, cs], preferred_element_type=F32)
                if first is None:
                    r = acc_v[:, cs] + r
                elif first is not True:
                    r = jnp.where(first, 0.0, acc_v[:, cs]) + r
                acc_v[:, cs] = r
                if blk == 0 and first is not True:
                    ob_v[0, :, cs] = r.astype(BF)

        def wait_all(cs):
            for c in cs:
                c.wait()

        for s in range(4):
            wait_all(start_copies(s))
            ks = pl.ds(s * KQ, KQ)
            for hp in range(2):
                cs = pl.ds(hp * 2 * DH, 2 * DH)
                r = jnp.dot(x_v[0, :, ks], wq_v[0, ks, cs], preferred_element_type=F32)
                if s > 0:
                    r = qp_v[:, cs] + r
                if s < 3:
                    qp_v[:, cs] = r
                else:
                    q_v[:, cs] = r.astype(BF)
        wait_all(start_copies(4))
        q = [load_qt(j) for j in range(NJ)]
        p0 = qk_t(0, 0, q[0])
        p1 = qk_t(0, 1, q[1])
        qproj(0, 1, 0)
        p2 = qk_t(0, 2, q[2])
        p3 = qk_t(0, 3, q[3])
        o0 = pv_t(0, 0, p0)
        o1 = pv_t(0, 1, p1)
        qproj(0, 1, 1)
        wait_all(start_copies(5))
        o2 = pv_t(0, 2, p2)
        o3 = pv_t(0, 3, p3)
        qproj(0, 1, 2)
        qproj(0, 1, 3)
        oproj(0, 0, jnp.concatenate([o0, o1, o2, o3], axis=0).astype(BF), True)

        def loop_a(g, c):
            @pl.when(g == NS - 1)
            def _():
                wait_all(cp_xb())

            @pl.when(g == 2)
            def _():
                wait_all(kv_rest())
            wait_all(step_copies(0, g))
            oproj(0, g, att_q(0, g), None)
            return c
        lax.fori_loop(1, NS, loop_a, 0)
        outs = out_copies()
        outs[0].start()

        def loop_b(g, c):
            wait_all(step_copies(1, g))
            oproj(1, g, att_q(1, g), g == 0)
            return c
        lax.fori_loop(0, NS - 1, loop_b, 0)

        g = NS - 1
        wait_all(step_copies(1, g))
        ps = [qk(g, h, load_q(h)) for h in range(G)]
        o0 = pv(g, 0, ps[0])
        o1 = pv(g, 1, ps[1])
        o01 = jnp.concatenate([o0, o1], axis=1).astype(BF)

        def oproj2(o2, hp, n):
            return jnp.dot(o2, wo_v[2 * NS - 1, pl.ds(hp * 2 * DH, 2 * DH), pl.ds(n * OC, OC)],
                           preferred_element_type=F32)
        o2 = pv(g, 2, ps[2])
        acc_v[:, pl.ds(0, OC)] += oproj2(o01, 0, 0)
        o3 = pv(g, 3, ps[3])
        for n in range(1, D // OC):
            acc_v[:, pl.ds(n * OC, OC)] += oproj2(o01, 0, n)
        o23 = jnp.concatenate([o2, o3], axis=1).astype(BF)
        for n in range(D // OC):
            cs = pl.ds(n * OC, OC)
            r = (acc_v[:, cs] + oproj2(o23, 1, n)).astype(BF)
            if n < D // OC - 1:
                ob_v[1, :, cs] = r
                outs[1 + n].start()
            else:
                for t in range(2):
                    ob_v[1, pl.ds(t * (M // 2), M // 2), cs] = r[t * (M // 2):(t + 1) * (M // 2)]
                    outs[1 + n + t].start()

    pl.run_scoped(main, pltpu.SemaphoreType.DMA((6,)), pltpu.SemaphoreType.DMA((2 * NS,)),
                  pltpu.SemaphoreType.REGULAR)
    for c in out_copies():
        c.wait()


@jax.jit
def pallas_concat_heads__gqa_block_cached__mha_block_cached__near_ridge_kernel(
    A_x, A_k_cache, A_v_cache, A_wq, A_wo, B_x, B_k_cache, B_v_cache, B_wq, B_wo,
):
    xa = A_x.reshape(M, D)
    xb = B_x.reshape(M, D)
    any_spec = pl.BlockSpec(memory_space=pl.ANY)
    out = pl.pallas_call(
        _kernel,
        out_shape=jax.ShapeDtypeStruct((M, 2 * D), BF),
        in_specs=[any_spec] * 10,
        out_specs=any_spec,
        scratch_shapes=[
            pltpu.VMEM((2, M, D), BF),
            pltpu.VMEM((2 * NS, D, CW), BF),
            pltpu.VMEM((2 * NS, CW, D), BF),
            pltpu.VMEM((NB, HKV, SK, DH), BF),
            pltpu.VMEM((NB, HKV, SK, DH), BF),
            pltpu.VMEM((NS, NB, G, SK, DH), BF),
            pltpu.VMEM((NS, NB, G, SK, DH), BF),
            pltpu.VMEM((M, CW), BF),
            pltpu.VMEM((M, CW), F32),
            pltpu.VMEM((M, D), F32),
            pltpu.VMEM((2, M, D), BF),
            pltpu.SemaphoreType.DMA((NOUT,)),
        ],
        compiler_params=pltpu.CompilerParams(vmem_limit_bytes=100 * 1024 * 1024),
    )(xa, A_k_cache, A_v_cache, A_wq, A_wo, xb, B_k_cache, B_v_cache, B_wq, B_wo)
    return out.reshape(NB, SQ, 2 * D)
```

```python
import jax
import jax.numpy as jnp
from jax import lax
from jax.experimental import pallas as pl
from jax.experimental.pallas import tpu as pltpu

NB, SQ, D = 16, 32, 1024
H, DH, SK = 32, 128, 32
HKV = 4
M = NB * SQ
G = 4
HS = 2 * G
NS = H // HS
CW = G * DH
SW = HS * DH
JB = 4
NJ = NB // JB
SCALE = DH ** -0.5
LOG2E = 1.4426950408889634
NT = (((1,), (1,)), ((), ()))
TN = (((0,), (0,)), ((), ()))
F32 = jnp.float32
BF = jnp.bfloat16
PAD = 128
PIECES = (
    ((0, 128, 0, 1024),),
    ((0, 128, 1024, 2048), (128, 256, 0, 512)),
    ((128, 256, 512, 2048), (256, 384, 0, 1536)),
    ((256, 384, 1536, 2048), (384, 640, 0, 2048)),
)
KL = 640
NP = len(PIECES)
OUT_B = ((0, M, 512, 256), (0, M, 768, 256), (0, M, 0, 256), (0, M, 256, 128),
         (0, M // 2, 384, 128), (M // 2, M // 2, 384, 128))


def _kernel(xa_h, ka_h, va_h, wqa_h, woa_h, xb_h, kb_h, vb_h, wqb_h, wob_h, out_h,
            x_v, wq_v, wo_v, ka_v, va_v, kb_v, vb_v, q_v, qp_v, acc_v, ob_v):
    wq_h = (wqa_h, wqb_h)
    wo_h = (woa_h, wob_h)
    cp = pltpu.make_async_copy

    def main(sem_s, sem_step, sem_out, bar):
        def barrier():
            pl.semaphore_signal(bar, 1)
            pl.semaphore_wait(bar, 1)

        def out_copies():
            cs = [cp(ob_v.at[0], out_h.at[:, pl.ds(0, D)], sem_out)]
            for r0, nr, c0, nc in OUT_B:
                cs.append(cp(ob_v.at[1, pl.ds(r0, nr), pl.ds(c0, nc)],
                             out_h.at[pl.ds(r0, nr), pl.ds(D + c0, nc)], sem_out))
            return cs

        def kva_copies(c, n, sem):
            hs = pl.ds(c, n)
            return [cp(ka_h.at[:, hs], ka_v.at[:, hs], sem), cp(va_h.at[:, hs], va_v.at[:, hs], sem)]

        def piece_copies(k0, k1, c0, c1, sem):
            ks = pl.ds(k0, k1 - k0)
            cs = []
            if c0 == 0:
                cs.append(cp(xa_h.at[:, ks], x_v.at[0, :, ks], sem))
            for s in range(2):
                lo, hi = max(c0, s * SW), min(c1, (s + 1) * SW)
                if lo < hi:
                    cs.append(cp(wqa_h.at[ks, pl.ds(lo, hi - lo)], wq_v.at[s, ks, pl.ds(lo - s * SW, hi - lo)], sem))
            return cs

        def cp_wo(blk, s, sem):
            return cp(wo_h[blk].at[pl.ds(s * SW, SW), :], wo_v.at[blk * NS + s, :, pl.ds(0, D)], sem)

        def start_copies(r):
            sem = sem_s.at[r]
            if r < NP:
                return [c for p in PIECES[r] for c in piece_copies(*p, sem)]
            if r == NP:
                return piece_copies(KL, D, 0, 2 * SW, sem) + kva_copies(0, 2, sem)
            return [cp_wo(0, 0, sem), cp_wo(0, 1, sem)]

        def step_copies(blk, s):
            i = blk * NS + s
            sem = sem_step.at[i]
            cs = [cp(wq_h[blk].at[:, pl.ds(s * SW, SW)], wq_v.at[i, :, pl.ds(0, SW)], sem)]
            if blk == 0:
                cs += kva_copies(s, 1, sem)
            else:
                cs.append(cp(kb_h.at[:, pl.ds(s * HS, HS)], kb_v.at[s], sem))
                cs.append(cp(vb_h.at[:, pl.ds(s * HS, HS)], vb_v.at[s], sem))
            cs.append(cp_wo(blk, s, sem))
            return cs

        def cp_xb():
            return [cp(xb_h, x_v.at[1, :, pl.ds(0, D)], sem_step.at[0])]

        for r in range(NP + 2):
            for c in start_copies(r):
                c.start()
            barrier()
        for i in range(2, 2 * NS):
            cs = step_copies(i // NS, i % NS)
            if i == NS:
                cs += cp_xb()
            for c in cs:
                c.start()
            if i < 2 * NS - 1:
                barrier()

        lane = lax.broadcasted_iota(jnp.int32, (SK, JB * SQ), 1)

        def softmax_t(d):
            m = jnp.max(d, axis=0, keepdims=True)
            e = jnp.exp2((d - m) * (SCALE * LOG2E))
            l = jnp.sum(e, axis=0, keepdims=True)
            return (e * pl.reciprocal(l, full_range=False)).astype(BF)

        def qk_m(s, u, t):
            h = u * G + t
            ps = []
            for j in range(NJ):
                q = q_v[pl.ds(j * JB * SQ, JB * SQ), pl.ds(h * DH, DH)]
                ks = kb_v[s, pl.ds(j * JB, JB), h].reshape(JB * SK, DH)
                st = lax.dot_general(ks, q, NT, preferred_element_type=F32)
                d = st[(JB - 1) * SK:]
                for r in range(JB - 2, -1, -1):
                    d = jnp.where(lane < (r + 1) * SQ, st[r * SK:(r + 1) * SK], d)
                ps.append(softmax_t(d).T)
            return ps

        def pv_m(s, u, t, ps):
            h = u * G + t
            os_ = []
            for j in range(NJ):
                for r in range(JB):
                    os_.append(jnp.dot(ps[j][r * SQ:(r + 1) * SQ], vb_v[s, j * JB + r, h],
                                       preferred_element_type=F32))
            return jnp.concatenate(os_, axis=0)

        def qk_g(s, u, j):
            ps = []
            for b in range(j * JB, (j + 1) * JB):
                qs = jnp.concatenate([q_v[pl.ds(b * SQ, SQ), pl.ds((u * G + h) * DH, DH)] for h in range(G)], axis=0)
                ps.append(softmax_t(lax.dot_general(ka_v[b, s], qs, NT, preferred_element_type=F32)))
            return ps

        def pv_g(s, u, j, ps):
            os_ = []
            for r in range(JB):
                o = lax.dot_general(ps[r], va_v[j * JB + r, s], TN, preferred_element_type=F32)
                os_.append(jnp.concatenate([o[h * SQ:(h + 1) * SQ] for h in range(G)], axis=1))
            return jnp.concatenate(os_, axis=0)

        def oproj(blk, os_, n, first, final, split=None):
            cs = pl.ds(n * DH, DH)
            r = None
            for i, u, o in os_:
                t = jnp.dot(o, wo_v[i, pl.ds(u * CW, CW), cs], preferred_element_type=F32)
                r = t if r is None else r + t
            if first is False:
                r = acc_v[:, cs] + r
            elif first is not True:
                r = jnp.where(first, 0.0, acc_v[:, cs]) + r
            acc_v[:, cs] = r
            if final and split is None:
                ob_v[blk, :, cs] = r.astype(BF)
            elif final:
                for t in range(2):
                    ob_v[blk, pl.ds(t * (M // 2), M // 2), cs] = r[t * (M // 2):(t + 1) * (M // 2)].astype(BF)
                    split(t)

        def wait_all(cs):
            for c in cs:
                c.wait()

        outs = out_copies()

        def step(blk, s, first):
            f_qk, f_pv = (qk_g, pv_g) if blk == 0 else (qk_m, pv_m)
            i = blk * NS + s

            def qproj(h):
                q_v[:, pl.ds(h * DH, DH)] = jnp.dot(x_v[blk, :, pl.ds(0, D)], wq_v[i, :, pl.ds(h * DH, DH)],
                                                    preferred_element_type=F32).astype(BF)

            def out_start(t):
                if blk == 1:
                    @pl.when(s == NS - 1)
                    def _():
                        outs[1 + t].start()

            for h in range(G + 1):
                qproj(h)
            p0 = f_qk(s, 0, 0)
            p1 = f_qk(s, 0, 1)
            qproj(G + 1)
            p2 = f_qk(s, 0, 2)
            p3 = f_qk(s, 0, 3)
            o0 = f_pv(s, 0, 0, p0)
            o1 = f_pv(s, 0, 1, p1)
            qproj(G + 2)
            o2 = f_pv(s, 0, 2, p2)
            o3 = f_pv(s, 0, 3, p3)
            qproj(G + 3)
            oa = (i, 0, jnp.concatenate([o0, o1, o2, o3], axis=blk).astype(BF))
            oproj(blk, [oa], 0, first, False)
            p0 = f_qk(s, 1, 0)
            p1 = f_qk(s, 1, 1)
            oproj(blk, [oa], 1, first, False)
            p2 = f_qk(s, 1, 2)
            p3 = f_qk(s, 1, 3)
            o0 = f_pv(s, 1, 0, p0)
            o1 = f_pv(s, 1, 1, p1)
            oproj(blk, [oa], 2, first, False)
            o2 = f_pv(s, 1, 2, p2)
            o3 = f_pv(s, 1, 3, p3)
            oproj(blk, [oa], 3, first, False)
            ob = (i, 1, jnp.concatenate([o0, o1, o2, o3], axis=blk).astype(BF))
            for n in range(4, 8):
                oproj(blk, [oa, ob], n, first, True)
                if n % 2 == 1:
                    out_start((n - 4) // 2)
            for n in range(4):
                oproj(blk, [ob], n, False, True,
                      split=(lambda t: out_start(4 + t)) if (n == 3 and blk == 1) else None)
                if n == 1:
                    out_start(2)
                if n == 2:
                    out_start(3)

        for r in range(NP):
            wait_all(start_copies(r))
            for k0, k1, c0, c1 in PIECES[r]:
                ks = pl.ds(k0, k1 - k0)
                for c in range(c0, c1, CW):
                    t = jnp.dot(x_v[0, :, ks], wq_v[c // SW, ks, pl.ds(c % SW, CW)], preferred_element_type=F32)
                    if k0 > 0:
                        t = qp_v[:, pl.ds(c, CW)] + t
                    qp_v[:, pl.ds(c, CW)] = t

        def qlast(u, half):
            rows = pl.ds(half * (M // 2), M // 2)
            ks = pl.ds(KL, D - KL)
            cs = pl.ds(u * CW, CW)
            t = jnp.dot(x_v[0, rows, ks], wq_v[u // 2, ks, pl.ds((u % 2) * CW, CW)], preferred_element_type=F32)
            q_v[rows, cs] = (qp_v[rows, cs] + t).astype(BF)

        wait_all(start_copies(NP))
        ps, os_ = {}, {}

        def do_qk(t):
            u, half = t // 2, t % 2
            for j in (2 * half, 2 * half + 1):
                ps[u, j] = qk_g(u // 2, u, j)

        def do_pv(t):
            u, half = t // 2, t % 2
            for j in (2 * half, 2 * half + 1):
                os_[u, j] = pv_g(u // 2, u, j, ps[u, j])

        for t in range(8):
            qlast(t // 2, t % 2)
            if t >= 1:
                do_qk(t - 1)
            if t >= 3:
                do_pv(t - 3)
        do_qk(7)
        do_pv(5)

        def o_of(u):
            return (u // 2, u % 2, jnp.concatenate([os_[u, j] for j in range(NJ)], axis=0).astype(BF))
        o3 = [o_of(u) for u in range(3)]
        wait_all(start_copies(NP + 1))
        oproj(0, o3, 0, True, False)
        do_pv(6)
        do_pv(7)
        oproj(0, o3, 1, True, False)
        ol = o_of(3)
        for n in range(2, 8):
            oproj(0, o3 + [ol], n, True, False)
        for n in range(2):
            oproj(0, [ol], n, False, False)

        def loop_a(s, c):
            wait_all(step_copies(0, s))
            step(0, s, False)
            return c
        lax.fori_loop(2, NS, loop_a, 0)
        outs[0].start()
        wait_all(cp_xb())

        def loop_b(s, c):
            wait_all(step_copies(1, s))
            step(1, s, s == 0)
            return c
        lax.fori_loop(0, NS, loop_b, 0)
        wait_all(outs)

    pl.run_scoped(main, pltpu.SemaphoreType.DMA((NP + 2,)), pltpu.SemaphoreType.DMA((2 * NS,)),
                  pltpu.SemaphoreType.DMA(()), pltpu.SemaphoreType.REGULAR)


@jax.jit
def pallas_concat_heads__gqa_block_cached__mha_block_cached__near_ridge_kernel(
    A_x, A_k_cache, A_v_cache, A_wq, A_wo, B_x, B_k_cache, B_v_cache, B_wq, B_wo,
):
    xa = A_x.reshape(M, D)
    xb = B_x.reshape(M, D)
    any_spec = pl.BlockSpec(memory_space=pl.ANY)
    out = pl.pallas_call(
        _kernel,
        out_shape=jax.ShapeDtypeStruct((M, 2 * D), BF),
        in_specs=[any_spec] * 10,
        out_specs=any_spec,
        scratch_shapes=[
            pltpu.VMEM((2, M, D + PAD), BF),
            pltpu.VMEM((2 * NS, D, SW + PAD), BF),
            pltpu.VMEM((2 * NS, SW, D + PAD), BF),
            pltpu.VMEM((NB, HKV, SK, DH), BF),
            pltpu.VMEM((NB, HKV, SK, DH), BF),
            pltpu.VMEM((NS, NB, HS, SK, DH), BF),
            pltpu.VMEM((NS, NB, HS, SK, DH), BF),
            pltpu.VMEM((M, 2 * SW + PAD), BF),
            pltpu.VMEM((M, 2 * SW), F32),
            pltpu.VMEM((M, D), F32),
            pltpu.VMEM((2, M, D), BF),
        ],
        compiler_params=pltpu.CompilerParams(vmem_limit_bytes=100 * 1024 * 1024),
    )(xa, A_k_cache, A_v_cache, A_wq, A_wo, xb, B_k_cache, B_v_cache, B_wq, B_wo)
    return out.reshape(NB, SQ, 2 * D)
```

```python
import jax
import jax.numpy as jnp
from jax import lax
from jax.experimental import pallas as pl
from jax.experimental.pallas import tpu as pltpu

NB, SQ, D = 16, 32, 1024
H, DH, SK = 32, 128, 32
HKV = 4
M = NB * SQ
G = 4
HS = 2 * G
NS = H // HS
CW = G * DH
SW = HS * DH
JB = 4
NJ = NB // JB
SCALE = DH ** -0.5
LOG2E = 1.4426950408889634
NT = (((1,), (1,)), ((), ()))
TN = (((0,), (0,)), ((), ()))
F32 = jnp.float32
BF = jnp.bfloat16
PAD = 128
PIECES = (
    ((0, 128, 0, 512),),
    ((0, 128, 512, 1536),),
    ((0, 128, 1536, 2048), (128, 256, 0, 1024)),
    ((128, 256, 1024, 2048), (256, 384, 0, 1536)),
    ((256, 384, 1536, 2048), (384, 640, 0, 2048)),
)
KL = 640
NP = len(PIECES)
OUT_B = ((0, M, 512, 256), (0, M, 768, 256), (0, M, 0, 256), (0, M, 256, 128),
         (0, 256, 384, 128), (256, 128, 384, 128), (384, 64, 384, 128), (448, 64, 384, 128))


def _kernel(xa_h, ka_h, va_h, wqa_h, woa_h, xb_h, kb_h, vb_h, wqb_h, wob_h, out_h,
            x_v, wq_v, wo_v, ka_v, va_v, kb_v, vb_v, q_v, qp_v, acc_v, ob_v):
    wq_h = (wqa_h, wqb_h)
    wo_h = (woa_h, wob_h)
    cp = pltpu.make_async_copy

    def main(sem_s, sem_step, sem_out, bar):
        def barrier():
            pl.semaphore_signal(bar, 1)
            pl.semaphore_wait(bar, 1)

        def out_copies():
            cs = [cp(ob_v.at[0], out_h.at[:, pl.ds(0, D)], sem_out)]
            for r0, nr, c0, nc in OUT_B:
                cs.append(cp(ob_v.at[1, pl.ds(r0, nr), pl.ds(c0, nc)],
                             out_h.at[pl.ds(r0, nr), pl.ds(D + c0, nc)], sem_out))
            return cs

        def kva_copies(c, n, sem):
            hs = pl.ds(c, n)
            return [cp(ka_h.at[:, hs], ka_v.at[:, hs], sem), cp(va_h.at[:, hs], va_v.at[:, hs], sem)]

        def piece_copies(k0, k1, c0, c1, sem):
            ks = pl.ds(k0, k1 - k0)
            cs = []
            if c0 == 0:
                cs.append(cp(xa_h.at[:, ks], x_v.at[0, :, ks], sem))
            for s in range(2):
                lo, hi = max(c0, s * SW), min(c1, (s + 1) * SW)
                if lo < hi:
                    cs.append(cp(wqa_h.at[ks, pl.ds(lo, hi - lo)],
                                 wq_v.at[s, ks, pl.ds(lo - s * SW, hi - lo)], sem))
            return cs

        def cp_wo(blk, s, sem):
            return cp(wo_h[blk].at[pl.ds(s * SW, SW), :], wo_v.at[blk * NS + s, :, pl.ds(0, D)], sem)

        def start_copies(r):
            sem = sem_s.at[r]
            if r < NP:
                return [c for p in PIECES[r] for c in piece_copies(*p, sem)]
            if r == NP:
                return piece_copies(KL, D, 0, 2 * SW, sem) + kva_copies(0, 2, sem)
            return [cp_wo(0, 0, sem), cp_wo(0, 1, sem)]

        def step_copies(blk, s):
            i = blk * NS + s
            sem = sem_step.at[i]
            cs = [cp(wq_h[blk].at[:, pl.ds(s * SW, SW)], wq_v.at[i, :, pl.ds(0, SW)], sem)]
            if blk == 0:
                cs += kva_copies(s, 1, sem)
            else:
                cs.append(cp(kb_h.at[:, pl.ds(s * HS, HS)], kb_v.at[s], sem))
                cs.append(cp(vb_h.at[:, pl.ds(s * HS, HS)], vb_v.at[s], sem))
            cs.append(cp_wo(blk, s, sem))
            return cs

        def cp_xb():
            return [cp(xb_h, x_v.at[1, :, pl.ds(0, D)], sem_step.at[0])]

        def wait_all(cs):
            for c in cs:
                c.wait()

        for r in range(NP + 2):
            for c in start_copies(r):
                c.start()
            barrier()
        for i in range(2, 2 * NS):
            cs = step_copies(i // NS, i % NS)
            if i == NS:
                cs += cp_xb()
            for c in cs:
                c.start()
            if i < 2 * NS - 1:
                barrier()

        lane = lax.broadcasted_iota(jnp.int32, (SK, JB * SQ), 1)
        outs = out_copies()

        def softmax_t(d):
            m = jnp.max(d, axis=0, keepdims=True)
            e = jnp.exp2((d - m) * (SCALE * LOG2E))
            l = jnp.sum(e, axis=0, keepdims=True)
            return (e * pl.reciprocal(l, full_range=False)).astype(BF)

        def qk_m(s, u, t):
            h = u * G + t
            ps = []
            for j in range(NJ):
                q = q_v[pl.ds(j * JB * SQ, JB * SQ), pl.ds(h * DH, DH)]
                ks = kb_v[s, pl.ds(j * JB, JB), h].reshape(JB * SK, DH)
                st = lax.dot_general(ks, q, NT, preferred_element_type=F32)
                d = st[(JB - 1) * SK:]
                for r in range(JB - 2, -1, -1):
                    d = jnp.where(lane < (r + 1) * SQ, st[r * SK:(r + 1) * SK], d)
                ps.append(softmax_t(d).T)
            return ps

        def pv_m(s, u, t, ps):
            h = u * G + t
            os_ = []
            for j in range(NJ):
                for r in range(JB):
                    os_.append(jnp.dot(ps[j][r * SQ:(r + 1) * SQ], vb_v[s, j * JB + r, h],
                                       preferred_element_type=F32))
            return jnp.concatenate(os_, axis=0)

        def qk_g(s, u, j):
            ps = []
            for b in range(j * JB, (j + 1) * JB):
                qs = jnp.concatenate(
                    [q_v[pl.ds(b * SQ, SQ), pl.ds((u * G + h) * DH, DH)] for h in range(G)], axis=0)
                ps.append(softmax_t(lax.dot_general(ka_v[b, s], qs, NT, preferred_element_type=F32)))
            return ps

        def pv_g(s, u, j, ps):
            os_ = []
            for r in range(JB):
                o = lax.dot_general(ps[r], va_v[j * JB + r, s], TN, preferred_element_type=F32)
                os_.append(jnp.concatenate([o[h * SQ:(h + 1) * SQ] for h in range(G)], axis=1))
            return jnp.concatenate(os_, axis=0)

        def oproj(blk, os_, n, first, final, split=None):
            cs = pl.ds(n * DH, DH)
            r = None
            for i, u, o in os_:
                t = jnp.dot(o, wo_v[i, pl.ds(u * CW, CW), cs], preferred_element_type=F32)
                r = t if r is None else r + t
            if first is False:
                r = acc_v[:, cs] + r
            elif first is not True:
                r = jnp.where(first, 0.0, acc_v[:, cs]) + r
            acc_v[:, cs] = r
            if final and split is None:
                ob_v[blk, :, cs] = r.astype(BF)
            elif final:
                for t, (r0, nr, _, _) in enumerate(OUT_B[4:]):
                    ob_v[blk, pl.ds(r0, nr), cs] = r[r0:r0 + nr].astype(BF)
                    split(t)

        def step(blk, s, first):
            f_qk, f_pv = (qk_g, pv_g) if blk == 0 else (qk_m, pv_m)
            i = blk * NS + s

            def qproj(h):
                q_v[:, pl.ds(h * DH, DH)] = jnp.dot(x_v[blk, :, pl.ds(0, D)], wq_v[i, :, pl.ds(h * DH, DH)],
                                                    preferred_element_type=F32).astype(BF)

            def out_start(t):
                if blk == 1:
                    @pl.when(s == NS - 1)
                    def _():
                        outs[1 + t].start()

            for h in range(G + 1):
                qproj(h)
            p0 = f_qk(s, 0, 0)
            p1 = f_qk(s, 0, 1)
            qproj(G + 1)
            p2 = f_qk(s, 0, 2)
            p3 = f_qk(s, 0, 3)
            o0 = f_pv(s, 0, 0, p0)
            o1 = f_pv(s, 0, 1, p1)
            qproj(G + 2)
            o2 = f_pv(s, 0, 2, p2)
            o3 = f_pv(s, 0, 3, p3)
            qproj(G + 3)
            oa = (i, 0, jnp.concatenate([o0, o1, o2, o3], axis=blk).astype(BF))
            oproj(blk, [oa], 0, first, False)
            p0 = f_qk(s, 1, 0)
            p1 = f_qk(s, 1, 1)
            oproj(blk, [oa], 1, first, False)
            p2 = f_qk(s, 1, 2)
            p3 = f_qk(s, 1, 3)
            o0 = f_pv(s, 1, 0, p0)
            o1 = f_pv(s, 1, 1, p1)
            oproj(blk, [oa], 2, first, False)
            o2 = f_pv(s, 1, 2, p2)
            o3 = f_pv(s, 1, 3, p3)
            oproj(blk, [oa], 3, first, False)
            ob = (i, 1, jnp.concatenate([o0, o1, o2, o3], axis=blk).astype(BF))
            for n in range(4, 8):
                oproj(blk, [oa, ob], n, first, True)
                if n % 2 == 1:
                    out_start((n - 4) // 2)
            for n in range(4):
                oproj(blk, [ob], n, False, True,
                      split=(lambda t: out_start(4 + t)) if (n == 3 and blk == 1) else None)
                if n == 1:
                    out_start(2)
                if n == 2:
                    out_start(3)

        def startup():
            for r in range(NP):
                wait_all(start_copies(r))
                for k0, k1, c0, c1 in PIECES[r]:
                    ks = pl.ds(k0, k1 - k0)
                    for c in range(c0, c1, CW):
                        t = jnp.dot(x_v[0, :, ks], wq_v[c // SW, ks, pl.ds(c % SW, CW)],
                                    preferred_element_type=F32)
                        if k0 > 0:
                            t = qp_v[:, pl.ds(c, CW)] + t
                        qp_v[:, pl.ds(c, CW)] = t

            def qlast(u, half):
                rows = pl.ds(half * (M // 2), M // 2)
                ks = pl.ds(KL, D - KL)
                cs = pl.ds(u * CW, CW)
                t = jnp.dot(x_v[0, rows, ks], wq_v[u // 2, ks, pl.ds((u % 2) * CW, CW)],
                            preferred_element_type=F32)
                q_v[rows, cs] = (qp_v[rows, cs] + t).astype(BF)

            wait_all(start_copies(NP))
            ps, os_ = {}, {}

            def do_qk(t):
                u, half = t // 2, t % 2
                for j in (2 * half, 2 * half + 1):
                    ps[u, j] = qk_g(u // 2, u, j)

            def do_pv(t):
                u, half = t // 2, t % 2
                for j in (2 * half, 2 * half + 1):
                    os_[u, j] = pv_g(u // 2, u, j, ps[u, j])

            def o_of(u):
                return (u // 2, u % 2, jnp.concatenate([os_[u, j] for j in range(NJ)], axis=0).astype(BF))

            for t in range(8):
                qlast(t // 2, t % 2)
                if t >= 1:
                    do_qk(t - 1)
                if t >= 3:
                    do_pv(t - 3)
            do_qk(7)
            do_pv(5)
            do_pv(6)
            o3 = [o_of(u) for u in range(3)]
            wait_all(start_copies(NP + 1))
            oproj(0, o3, 0, True, False)
            do_pv(7)
            oproj(0, o3, 1, True, False)
            ol = o_of(3)
            for n in range(2, 8):
                oproj(0, o3 + [ol], n, True, False)
            for n in range(2):
                oproj(0, [ol], n, False, False)

        def loop_a(s, c):
            wait_all(step_copies(0, s))
            step(0, s, False)
            return c

        def loop_b(s, c):
            wait_all(step_copies(1, s))
            step(1, s, s == 0)
            return c

        def phase(t, c):
            @pl.when(t == 1)
            def _():
                startup()
                lax.fori_loop(2, NS, loop_a, 0)
                outs[0].start()
                wait_all(cp_xb())
                lax.fori_loop(0, NS, loop_b, 0)
            return c
        lax.fori_loop(0, 2, phase, 0)
        wait_all(outs)

    pl.run_scoped(main, pltpu.SemaphoreType.DMA((NP + 2,)), pltpu.SemaphoreType.DMA((2 * NS,)),
                  pltpu.SemaphoreType.DMA(()), pltpu.SemaphoreType.REGULAR)


@jax.jit
def pallas_concat_heads__gqa_block_cached__mha_block_cached__near_ridge_kernel(
    A_x: jax.Array,
    A_k_cache: jax.Array,
    A_v_cache: jax.Array,
    A_wq: jax.Array,
    A_wo: jax.Array,
    B_x: jax.Array,
    B_k_cache: jax.Array,
    B_v_cache: jax.Array,
    B_wq: jax.Array,
    B_wo: jax.Array,
):
    xa = A_x.reshape(M, D)
    xb = B_x.reshape(M, D)
    any_spec = pl.BlockSpec(memory_space=pl.ANY)
    out = pl.pallas_call(
        _kernel,
        out_shape=jax.ShapeDtypeStruct((M, 2 * D), BF),
        in_specs=[any_spec] * 10,
        out_specs=any_spec,
        scratch_shapes=[
            pltpu.VMEM((2, M, D + PAD), BF),
            pltpu.VMEM((2 * NS, D, SW + PAD), BF),
            pltpu.VMEM((2 * NS, SW, D + PAD), BF),
            pltpu.VMEM((NB, HKV, SK, DH), BF),
            pltpu.VMEM((NB, HKV, SK, DH), BF),
            pltpu.VMEM((NS, NB, HS, SK, DH), BF),
            pltpu.VMEM((NS, NB, HS, SK, DH), BF),
            pltpu.VMEM((M, 2 * SW + PAD), BF),
            pltpu.VMEM((M, 2 * SW), F32),
            pltpu.VMEM((M, D), F32),
            pltpu.VMEM((2, M, D), BF),
        ],
        compiler_params=pltpu.CompilerParams(vmem_limit_bytes=100 * 1024 * 1024),
    )(xa, A_k_cache, A_v_cache, A_wq, A_wo, xb, B_k_cache, B_v_cache, B_wq, B_wo)
    return out.reshape(NB, SQ, 2 * D)
```
